```python
import os as _os
_os.environ.setdefault("JAX_PLATFORMS", "cpu")
import jax
import jax.numpy as jnp

def _softmax(x, axis=-1):
    return jax.nn.softmax(x, axis=axis)
def _gelu(x):
    return jax.nn.gelu(x, approximate=True)
def _silu(x):
    return jax.nn.silu(x)
def _sigmoid(x):
    return jax.nn.sigmoid(x)
def _layernorm(x, axis=-1, eps=1e-5):
    m = jnp.mean(x, axis=axis, keepdims=True)
    v = jnp.var(x, axis=axis, keepdims=True)
    return (x - m) / jnp.sqrt(v + eps)
def _scatter_add(tgt, idx, src, axis=0):
    return tgt.at[idx].add(src)
def _segment_sum(src, seg, n):
    return jax.ops.segment_sum(src, seg, n)
class _Rng:
    def __init__(self, key):
        self._k = key
    def _next(self):
        self._k, sub = jax.random.split(self._k)
        return sub
    def normal(self, shape):
        return jax.random.normal(self._next(), shape, dtype=jnp.bfloat16)
    def randint(self, lo, hi, shape):
        return jax.random.randint(self._next(), shape, lo, hi, dtype=jnp.int32)
    def uniform(self, shape, lo=0.0, hi=1.0):
        return jax.random.uniform(self._next(), shape, jnp.bfloat16, lo, hi)
    def permutation(self, n):
        return jax.random.permutation(self._next(), n)


kernel_name = 'standalone__gqa_block_cached__near_ridge'

def setup_inputs():
    _rng = _Rng(jax.random.key(int.from_bytes(__import__("os").urandom(4), "little")))
    _w = (lambda a: (lambda t: t.astype(jnp.bfloat16) if jnp.issubdtype(t.dtype, jnp.floating) else t)(jnp.asarray(a)))
    B, Sq, D = 8, 96, 448
    Hq, Hkv, Sk, Dh = 16, 8, 2048, 256
    assert Hq % Hkv == 0, (Hq, Hkv)
    return {
        "x": _w((lambda *s: _rng.normal(s) * 0.8)(B, Sq, D)),
        "k_cache": _w((lambda *s: _rng.normal(s) * 0.8)(B, Hkv, Sk, Dh)),
        "v_cache": _w((lambda *s: _rng.normal(s) * 0.05)(B, Hkv, Sk, Dh)),
        "wq": _w((lambda *s: _rng.normal(s) * 0.8)(D, Hq * Dh) * (D ** -0.5)),
        "wo": _w((lambda *s: _rng.normal(s) * 0.05)(Hq * Dh, D) * ((Hq * Dh) ** -0.5)),
    }

def reference(x, k_cache, v_cache, wq, wo):
    B, Sq, D = x.shape
    Hq, Dh = 16, 256
    Hkv = k_cache.shape[1]
    rep = Hq // Hkv
    q = (lambda x, *d: x.transpose(*d))((x @ wq).reshape(B, Sq, Hq, Dh), 0, 2, 1, 3)
    k = jnp.repeat(k_cache, rep, axis=1)
    v = jnp.repeat(v_cache, rep, axis=1)
    scores = jnp.einsum("bhqd,bhkd->bhqk", q, k) * (Dh ** -0.5)
    p = _softmax(scores, axis=-1)
    o = jnp.einsum("bhqk,bhkd->bhqd", p, v)
    return (lambda x, *d: x.transpose(*d))(o, 0, 2, 1, 3).reshape(B, Sq, Hq * Dh) @ wo
```

```python
import functools
import jax
import jax.numpy as jnp
from jax import lax
import jax.experimental.pallas as pl
import jax.experimental.pallas.tpu as pltpu

B, SQ, D = 8, 96, 448
HQ, HKV, SK, DH = 16, 8, 2048, 256
REP = HQ // HKV
GW = REP * DH
M = REP * SQ
NT = (((1,), (1,)), ((), ()))
LOG2E = 1.4426950408889634


def make_kernel(nbuf=4, ck=256, nodma=False, order=0, ahead=0, exp2=False, mpass=False, nobc=True,
                unroll2=False, fin_late=False, flags=None):
    nsteps = HKV * B
    nch = SK // ck
    assert nbuf & (nbuf - 1) == 0 or not unroll2
    pow2 = nbuf & (nbuf - 1) == 0

    def modn(x):
        return (x & (nbuf - 1)) if pow2 else lax.rem(x, nbuf)

    def kern(x_hbm, k_hbm, v_hbm, wq_hbm, wo_hbm, out_hbm,
             x_v, wq_v, wo_v, kbuf, vbuf, q_scr, o_scr, acc, out_v, s_scr, m_scr, l_scr, pv_scr,
             k_sems, v_sems, w_sems, misc_sems):
        def k_copy(step):
            slot = modn(step)
            return pltpu.make_async_copy(k_hbm.at[step & (B - 1), step >> 3], kbuf.at[slot], k_sems.at[slot])

        def v_copy(step):
            slot = modn(step)
            return pltpu.make_async_copy(v_hbm.at[step & (B - 1), step >> 3], vbuf.at[slot], v_sems.at[slot])

        def wq_copy(h):
            return pltpu.make_async_copy(wq_hbm.at[:, pl.ds(pl.multiple_of(h * GW, GW), GW)], wq_v.at[h & 1], w_sems.at[0, h & 1])

        def wo_copy(h):
            return pltpu.make_async_copy(wo_hbm.at[:, pl.ds(pl.multiple_of(h * GW, GW), GW)], wo_v.at[h & 1], w_sems.at[1, h & 1])

        def q_proj(h):
            xv = x_v[...].reshape(B * SQ, D)
            sc = (DH ** -0.5)
            q = jnp.dot(xv, wq_v[h & 1], preferred_element_type=jnp.float32) * sc
            q = q.astype(jnp.bfloat16)
            for b in range(B):
                for r in range(REP):
                    q_scr[(h & 1) * B + b, r * SQ:(r + 1) * SQ, :] = q[b * SQ:(b + 1) * SQ, r * DH:(r + 1) * DH]

        def qk_chunk(step, slot, c, par):
            s = lax.dot_general(q_scr[step & (2 * B - 1)], kbuf[slot, c * ck:(c + 1) * ck, :], NT,
                                preferred_element_type=jnp.float32)
            s_scr[par, :, c * ck:(c + 1) * ck] = s
            if not mpass:
                mx = s[:, 0:128]
                for j in range(1, ck // 128):
                    mx = jnp.maximum(mx, s[:, j * 128:(j + 1) * 128])
                if c == 0:
                    m_scr[par] = mx
                else:
                    m_scr[par] = jnp.maximum(m_scr[par], mx)

        def exp_chunk(par, c, m):
            d = s_scr[par, :, c * ck:(c + 1) * ck] - m
            p = jnp.exp2(d * LOG2E) if exp2 == 1 else jnp.exp(d)
            ls = p[:, 0:128]
            for j in range(1, ck // 128):
                ls = ls + p[:, j * 128:(j + 1) * 128]
            if c == 0:
                l_scr[...] = ls
            else:
                l_scr[...] += ls
            return p.astype(jnp.bfloat16)

        def pv_chunk(p, vslot, c):
            pv = jnp.dot(p, vbuf[vslot, c * ck:(c + 1) * ck, :], preferred_element_type=jnp.float32)
            if c == 0:
                pv_scr[...] = pv
            else:
                pv_scr[...] += pv

        def finalize(step):
            l = jnp.sum(l_scr[...], axis=-1, keepdims=True)
            o = (pv_scr[...] / l).astype(jnp.bfloat16)
            row = pl.multiple_of((step & (B - 1)) * SQ, SQ)
            for r in range(REP):
                o_scr[pl.ds(row, SQ), r * DH:(r + 1) * DH] = o[r * SQ:(r + 1) * SQ, :]

        def body(step, par, wpar, do_next):
            ns = nbuf
            vslot = modn(step) if not nodma else 0
            kslot = modn(step + 1) if not nodma else 1
            if mpass:
                mx = s_scr[par, :, 0:128]
                for j in range(1, SK // 128):
                    mx = jnp.maximum(mx, s_scr[par, :, j * 128:(j + 1) * 128])
            else:
                mx = m_scr[par]
            m = jnp.max(mx, axis=-1, keepdims=True)
            ps = {}
            for c in range(min(ahead, nch)):
                ps[c] = exp_chunk(par, c, m)
            for c in range(nch):
                if do_next and order == 0:
                    qk_chunk(step + 1, kslot, c, wpar)
                if c + ahead < nch:
                    ps[c + ahead] = exp_chunk(par, c + ahead, m)
                if do_next and order == 2:
                    qk_chunk(step + 1, kslot, c, wpar)
                pv_chunk(ps.pop(c), vslot, c)
                if do_next and order == 1:
                    qk_chunk(step + 1, kslot, c, wpar)
            finalize(step)

        def dma_part(step, last):
            nx = step + nbuf - 1
            if nodma:
                return
            @pl.when(nx < nsteps)
            def _():
                v_copy(nx).start()

            @pl.when(nx + 1 < nsteps)
            def _():
                k_copy(nx + 1).start()

            v_copy(step).wait()
            if not last:
                k_copy(step + 1).wait()

        x_copy = pltpu.make_async_copy(x_hbm, x_v, misc_sems.at[0])
        x_copy.start()
        wq_copy(0).start()
        k_copy(0).start()
        wq_copy(1).start()
        for s in range(nbuf - 1):
            v_copy(s).start()
            k_copy(s + 1).start()
        wo_copy(0).start()
        acc[...] = jnp.zeros_like(acc)
        x_copy.wait()
        wq_copy(0).wait()
        q_proj(0)
        k_copy(0).wait()
        if nodma:
            for s in range(nbuf - 1):
                v_copy(s).wait()
                k_copy(s + 1).wait()
        for c in range(nch):
            qk_chunk(0, 0, c, 0)

        def group(h, carry):
            @pl.when(h + 1 < HKV)
            def _():
                wq_copy(h + 1).wait()
                q_proj(h + 1)

            @pl.when(h + 2 < HKV)
            def _():
                wq_copy(h + 2).start()

            if not unroll2:
                def step_fn(b, c):
                    step = h * B + b
                    rd, wr = c

                    @pl.when(step < nsteps - 1)
                    def _():
                        dma_part(step, False)
                        body(step, rd, wr, True)

                    @pl.when(step == nsteps - 1)
                    def _():
                        dma_part(step, True)
                        body(step, rd, wr, False)

                    return (wr, rd)
                carry = lax.fori_loop(0, B, step_fn, carry)
            else:
                def step_fn(b2, c):
                    step = h * B + 2 * b2
                    dma_part(step, False)
                    body(step, 0, True)

                    @pl.when(step + 1 < nsteps - 1)
                    def _():
                        dma_part(step + 1, False)
                        body(step + 1, 1, True)

                    @pl.when(step + 1 == nsteps - 1)
                    def _():
                        dma_part(step + 1, True)
                        body(step + 1, 1, False)

                    return c
                lax.fori_loop(0, B // 2, step_fn, 0)

            wo_copy(h).wait()
            part = lax.dot_general(o_scr[...], wo_v[h & 1], NT, preferred_element_type=jnp.float32)
            acc[...] += part

            @pl.when(h + 1 < HKV)
            def _():
                wo_copy(h + 1).start()

            return carry

        lax.fori_loop(0, HKV, group, (jnp.int32(0), jnp.int32(1)))
        out_v[...] = acc[...].astype(jnp.bfloat16).reshape(B, SQ, D)
        oc = pltpu.make_async_copy(out_v, out_hbm, misc_sems.at[1])
        oc.start()
        oc.wait()

    cp = dict(vmem_limit_bytes=100 * 1024 * 1024)
    if nobc:
        cp["disable_bounds_checks"] = True
    if flags:
        cp["flags"] = {f: True for f in flags.split("+")}

    def call(x, k_cache, v_cache, wq, wo):
        return pl.pallas_call(
            kern,
            out_shape=jax.ShapeDtypeStruct((B, SQ, D), jnp.bfloat16),
            in_specs=[pl.BlockSpec(memory_space=pltpu.MemorySpace.HBM)] * 5,
            out_specs=pl.BlockSpec(memory_space=pltpu.MemorySpace.HBM),
            scratch_shapes=[
                pltpu.VMEM((B, SQ, D), jnp.bfloat16),
                pltpu.VMEM((2, D, GW), jnp.bfloat16),
                pltpu.VMEM((2, D, GW), jnp.bfloat16),
                pltpu.VMEM((nbuf, SK, DH), jnp.bfloat16),
                pltpu.VMEM((nbuf, SK, DH), jnp.bfloat16),
                pltpu.VMEM((2 * B, M, DH), jnp.bfloat16),
                pltpu.VMEM((B * SQ, GW), jnp.bfloat16),
                pltpu.VMEM((B * SQ, D), jnp.float32),
                pltpu.VMEM((B, SQ, D), jnp.bfloat16),
                pltpu.VMEM((2, M, SK), jnp.float32),
                pltpu.VMEM((2, M, 128), jnp.float32),
                pltpu.VMEM((M, 128), jnp.float32),
                pltpu.VMEM((M, DH), jnp.float32),
                pltpu.SemaphoreType.DMA((nbuf,)),
                pltpu.SemaphoreType.DMA((nbuf,)),
                pltpu.SemaphoreType.DMA((2, 2)),
                pltpu.SemaphoreType.DMA((2,)),
            ],
            compiler_params=pltpu.CompilerParams(**cp),
        )(x, k_cache, v_cache, wq, wo.T)

    return call


@jax.jit
def pallas_standalone__gqa_block_cached__near_ridge_kernel(x, k_cache, v_cache, wq, wo):
    return make_kernel(order=2, ahead=1)(x, k_cache, v_cache, wq, wo)
```

```python
import jax
import jax.numpy as jnp
from jax import lax
import jax.experimental.pallas as pl
import jax.experimental.pallas.tpu as pltpu

_HQ, _DH = 16, 256
_NBUF = 4
_CK = 256
_NT = (((1,), (1,)), ((), ()))


@jax.jit
def pallas_standalone__gqa_block_cached__near_ridge_kernel(
    x: jax.Array,
    k_cache: jax.Array,
    v_cache: jax.Array,
    wq: jax.Array,
    wo: jax.Array,
):
    B, SQ, D = x.shape
    HKV, SK = k_cache.shape[1], k_cache.shape[2]
    DH = _DH
    REP = _HQ // HKV
    GW = REP * DH
    M = REP * SQ
    nbuf, ck = _NBUF, _CK
    nsteps = HKV * B
    nch = SK // ck
    lasth = HKV - 1
    logb = B.bit_length() - 1
    assert B == 1 << logb and B % 2 == 0 and HKV >= 2
    assert SK % ck == 0 and ck % 128 == 0 and SQ % 16 == 0
    assert nbuf & (nbuf - 1) == 0 and nbuf <= B

    def kernel(
        x_hbm, k_hbm, v_hbm, wq_hbm, wo_hbm, out_hbm,
        x_v, wq_v, wo_v, kbuf, vbuf, q_scr, o_scr, acc, out_v,
        s_scr, m_scr, l_scr, pv_scr, m_fin,
        k_sems, v_sems, w_sems, x_sem, o_sems,
    ):
        def k_copy(step):
            slot = step & (nbuf - 1)
            return pltpu.make_async_copy(
                k_hbm.at[step & (B - 1), step >> logb], kbuf.at[slot], k_sems.at[slot])

        def v_copy(step):
            slot = step & (nbuf - 1)
            return pltpu.make_async_copy(
                v_hbm.at[step & (B - 1), step >> logb], vbuf.at[slot], v_sems.at[slot])

        def wq_copy(h):
            return pltpu.make_async_copy(
                wq_hbm.at[:, pl.ds(pl.multiple_of(h * GW, GW), GW)],
                wq_v.at[h & 1], w_sems.at[0, h & 1])

        def wo_copy(h):
            return pltpu.make_async_copy(
                wo_hbm.at[:, pl.ds(pl.multiple_of(h * GW, GW), GW)],
                wo_v.at[h & 1], w_sems.at[1, h & 1])

        def out_copy(b):
            return pltpu.make_async_copy(out_v.at[b], out_hbm.at[b], o_sems.at[b])

        def q_proj(h):
            xv = x_v[...].reshape(B * SQ, D)
            q = jnp.dot(xv, wq_v[h & 1], preferred_element_type=jnp.float32) * (DH ** -0.5)
            q = q.astype(jnp.bfloat16)
            for b in range(B):
                for r in range(REP):
                    q_scr[(h & 1) * B + b, r * SQ:(r + 1) * SQ, :] = (
                        q[b * SQ:(b + 1) * SQ, r * DH:(r + 1) * DH])

        def qk_chunk(step, c, par, tok=None):
            s = lax.dot_general(
                q_scr[step & (2 * B - 1)], kbuf[step & (nbuf - 1), c * ck:(c + 1) * ck, :],
                _NT, preferred_element_type=jnp.float32)
            s_scr[par, :, c * ck:(c + 1) * ck] = s
            if tok is not None:
                m_fin[tok, 0:8, :] = s[0:8, 0:128]
            mx = s[:, 0:128]
            for j in range(1, ck // 128):
                mx = jnp.maximum(mx, s[:, j * 128:(j + 1) * 128])
            if c == 0:
                m_scr[par] = mx
            else:
                m_scr[par] = jnp.maximum(m_scr[par], mx)

        def exp_chunk(par, c, m):
            d = jnp.concatenate(
                [s_scr[par, :, c * ck + j * 128:c * ck + (j + 1) * 128] - m
                 for j in range(ck // 128)], axis=1)
            p = jnp.exp(d)
            ls = p[:, 0:128]
            for j in range(1, ck // 128):
                ls = ls + p[:, j * 128:(j + 1) * 128]
            if c == 0:
                l_scr[...] = ls
            else:
                l_scr[...] += ls
            return p.astype(jnp.bfloat16)

        def pv_chunk(step, p, c):
            pv = jnp.dot(p, vbuf[step & (nbuf - 1), c * ck:(c + 1) * ck, :],
                         preferred_element_type=jnp.float32)
            if c == 0:
                pv_scr[...] = pv
            else:
                pv_scr[...] += pv

        def prefetch(step, guarded):
            nx = step + nbuf - 1
            if guarded:
                pl.when(nx < nsteps)(lambda: v_copy(nx).start())
                pl.when(nx + 1 < nsteps)(lambda: k_copy(nx + 1).start())
            else:
                v_copy(nx).start()
                k_copy(nx + 1).start()

        def attend(step, par, do_next, rd, wr, guarded=False):
            v_copy(step).wait()
            if do_next:
                k_copy(step + 1).wait()
                prefetch(step, guarded)
            m = jnp.max(m_scr[par], axis=-1, keepdims=True)
            m_fin[rd] = jnp.broadcast_to(m, (M, 128))
            p = exp_chunk(par, 0, m_fin[rd])
            for c in range(nch):
                if do_next:
                    qk_chunk(step + 1, c, 1 - par, wr)
                p_next = exp_chunk(par, c + 1, m_fin[rd]) if c + 1 < nch else None
                pv_chunk(step, p, c)
                p = p_next
            l = jnp.sum(l_scr[...], axis=-1, keepdims=True)
            return (pv_scr[...] / l).astype(jnp.bfloat16)

        def store_o(step, o):
            row = pl.multiple_of((step & (B - 1)) * SQ, SQ)
            for r in range(REP):
                o_scr[pl.ds(row, SQ), r * DH:(r + 1) * DH] = o[r * SQ:(r + 1) * SQ, :]

        def final_rows(b, o):
            row = pl.multiple_of(b * SQ, SQ)
            oc = jnp.concatenate([o[r * SQ:(r + 1) * SQ, :] for r in range(REP)], axis=1)
            part = lax.dot_general(oc, wo_v[lasth & 1], _NT,
                                   preferred_element_type=jnp.float32)
            out_v[b] = (acc[pl.ds(row, SQ), :] + part).astype(jnp.bfloat16)
            out_copy(b).start()

        x_copy = pltpu.make_async_copy(x_hbm, x_v, x_sem)
        x_copy.start()
        wq_copy(0).start()
        k_copy(0).start()
        acc[...] = jnp.zeros_like(acc)
        x_copy.wait()
        wq_copy(0).wait()
        wq_copy(1).start()
        for s in range(nbuf - 1):
            v_copy(s).start()
            k_copy(s + 1).start()
        wo_copy(0).start()
        q_proj(0)
        k_copy(0).wait()
        for c in range(nch):
            qk_chunk(0, c, 0)

        def group(h, carry):
            wq_copy(h + 1).wait()
            q_proj(h + 1)
            pl.when(h + 2 < HKV)(lambda: wq_copy(h + 2).start())
            wo_copy(h + 1).start()

            def pair(bu, c):
                rd, wr = c
                for u in range(2):
                    step = h * B + 2 * bu + u
                    store_o(step, attend(step, u, True, rd, wr))
                    rd, wr = wr, rd
                return (c[1], c[0])

            carry = lax.fori_loop(0, B // 2, pair, carry)
            wo_copy(h).wait()
            acc[...] += lax.dot_general(o_scr[...], wo_v[h & 1], _NT,
                                        preferred_element_type=jnp.float32)
            return carry

        carry = lax.fori_loop(0, HKV - 1, group, (jnp.int32(0), jnp.int32(1)))

        wo_copy(lasth).wait()

        def last_pair(bu, c):
            rd, wr = c
            for u in range(2):
                step = lasth * B + 2 * bu + u

                def run(step=step, u=u, rd=rd, wr=wr):
                    o = attend(step, u, True, rd, wr, guarded=True)
                    final_rows(step & (B - 1), o)

                if u == 0:
                    run()
                else:
                    pl.when(step < nsteps - 1)(run)
                rd, wr = wr, rd
            return (c[1], c[0])

        rd, wr = lax.fori_loop(0, B // 2, last_pair, carry)
        final_rows(B - 1, attend(nsteps - 1, 1, False, rd, wr))
        for b in range(B):
            out_copy(b).wait()

    hbm = pl.BlockSpec(memory_space=pltpu.MemorySpace.HBM)
    return pl.pallas_call(
        kernel,
        out_shape=jax.ShapeDtypeStruct((B, SQ, D), jnp.bfloat16),
        in_specs=[hbm] * 5,
        out_specs=hbm,
        scratch_shapes=[
            pltpu.VMEM((B, SQ, D), jnp.bfloat16),
            pltpu.VMEM((2, D, GW), jnp.bfloat16),
            pltpu.VMEM((2, D, GW), jnp.bfloat16),
            pltpu.VMEM((nbuf, SK, DH), jnp.bfloat16),
            pltpu.VMEM((nbuf, SK, DH), jnp.bfloat16),
            pltpu.VMEM((2 * B, M, DH), jnp.bfloat16),
            pltpu.VMEM((B * SQ, GW), jnp.bfloat16),
            pltpu.VMEM((B * SQ, D), jnp.float32),
            pltpu.VMEM((B, SQ, D), jnp.bfloat16),
            pltpu.VMEM((2, M, SK), jnp.float32),
            pltpu.VMEM((2, M, 128), jnp.float32),
            pltpu.VMEM((M, 128), jnp.float32),
            pltpu.VMEM((M, DH), jnp.float32),
            pltpu.VMEM((2, M, 128), jnp.float32),
            pltpu.SemaphoreType.DMA((nbuf,)),
            pltpu.SemaphoreType.DMA((nbuf,)),
            pltpu.SemaphoreType.DMA((2, 2)),
            pltpu.SemaphoreType.DMA(()),
            pltpu.SemaphoreType.DMA((B,)),
        ],
        compiler_params=pltpu.CompilerParams(vmem_limit_bytes=64 * 1024 * 1024),
    )(x, k_cache, v_cache, wq, wo.T)
```

```python
import jax
import jax.numpy as jnp
from jax import lax
import jax.experimental.pallas as pl
import jax.experimental.pallas.tpu as pltpu

_HQ, _DH = 16, 256
_NBUF = 8
_LK, _LV = 3, 5
_NPK = 64
_NF = 2
_CK = 256
_NT = (((1,), (1,)), ((), ()))


@jax.jit
def pallas_standalone__gqa_block_cached__near_ridge_kernel(
    x: jax.Array,
    k_cache: jax.Array,
    v_cache: jax.Array,
    wq: jax.Array,
    wo: jax.Array,
):
    B, SQ, D = x.shape
    HKV, SK = k_cache.shape[1], k_cache.shape[2]
    DH = _DH
    REP = _HQ // HKV
    GW = REP * DH
    M = REP * SQ
    nbuf, ck = _NBUF, _CK
    nsteps = HKV * B
    nch = SK // ck
    lasth = HKV - 1
    logb = B.bit_length() - 1
    assert B == 1 << logb and B % 2 == 0 and HKV >= 2
    assert SK % ck == 0 and ck % 128 == 0 and SQ % 16 == 0
    assert nbuf & (nbuf - 1) == 0 and max(_LK, _LV) < nbuf
    assert _NF + _LV + 1 <= B and _NPK % nch == 0 and SK % (16 * _NPK) == 0

    def kernel(
        x_hbm, k_hbm, v_hbm, wq_hbm, wo_hbm, out_hbm,
        x_v, wq_v, wo_v, kbuf, vbuf, q_scr, o_scr, acc, out_v,
        s_scr, m_scr, l_scr, pv_scr, m_fin,
        k_sems, v_sems, w_sems, x_sem, o_sems,
    ):
        def k_copy(step):
            slot = step & (nbuf - 1)
            return pltpu.make_async_copy(
                k_hbm.at[step & (B - 1), step >> logb], kbuf.at[slot], k_sems.at[slot])

        def k_piece(step, j):
            slot = step & (nbuf - 1)
            rows = pl.ds(j * (SK // _NPK), SK // _NPK)
            return pltpu.make_async_copy(
                k_hbm.at[step & (B - 1), step >> logb, rows], kbuf.at[slot, rows],
                k_sems.at[slot])

        def k_wait(step):
            slot = step & (nbuf - 1)
            pltpu.make_async_copy(kbuf.at[slot], kbuf.at[slot], k_sems.at[slot]).wait()

        def v_copy(step):
            slot = step & (nbuf - 1)
            return pltpu.make_async_copy(
                v_hbm.at[step & (B - 1), step >> logb], vbuf.at[slot], v_sems.at[slot])

        def wq_copy(h):
            return pltpu.make_async_copy(
                wq_hbm.at[:, pl.ds(pl.multiple_of(h * GW, GW), GW)],
                wq_v.at[h & 1], w_sems.at[0, h & 1])

        def wo_copy(h):
            return pltpu.make_async_copy(
                wo_hbm.at[:, pl.ds(pl.multiple_of(h * GW, GW), GW)],
                wo_v.at[h & 1], w_sems.at[1, h & 1])

        def out_copy(b):
            return pltpu.make_async_copy(out_v.at[b], out_hbm.at[b], o_sems.at[b])

        def q_proj(h):
            xv = x_v[...].reshape(B * SQ, D)
            q = jnp.dot(xv, wq_v[h & 1], preferred_element_type=jnp.float32) * (DH ** -0.5)
            q = q.astype(jnp.bfloat16)
            for b in range(B):
                for r in range(REP):
                    q_scr[(h & 1) * B + b, r * SQ:(r + 1) * SQ, :] = (
                        q[b * SQ:(b + 1) * SQ, r * DH:(r + 1) * DH])

        def qk_chunk(step, c, par, tok=None):
            s = lax.dot_general(
                q_scr[step & (2 * B - 1)], kbuf[step & (nbuf - 1), c * ck:(c + 1) * ck, :],
                _NT, preferred_element_type=jnp.float32)
            s_scr[par, :, c * ck:(c + 1) * ck] = s
            if tok is not None:
                m_fin[tok, 0:8, :] = s[0:8, 0:128]
            mx = s[:, 0:128]
            for j in range(1, ck // 128):
                mx = jnp.maximum(mx, s[:, j * 128:(j + 1) * 128])
            if c == 0:
                m_scr[par] = mx
            else:
                m_scr[par] = jnp.maximum(m_scr[par], mx)

        def exp_chunk(par, c, m):
            d = jnp.concatenate(
                [s_scr[par, :, c * ck + j * 128:c * ck + (j + 1) * 128] - m
                 for j in range(ck // 128)], axis=1)
            p = jnp.exp(d)
            ls = p[:, 0:128]
            for j in range(1, ck // 128):
                ls = ls + p[:, j * 128:(j + 1) * 128]
            if c == 0:
                l_scr[...] = ls
            else:
                l_scr[...] += ls
            return p.astype(jnp.bfloat16)

        def pv_chunk(step, p, c):
            pv = jnp.dot(p, vbuf[step & (nbuf - 1), c * ck:(c + 1) * ck, :],
                         preferred_element_type=jnp.float32)
            if c == 0:
                pv_scr[...] = pv
            else:
                pv_scr[...] += pv

        def prefetch_v(step, guarded):
            nx = step + _LV
            if guarded:
                pl.when(nx < nsteps)(lambda: v_copy(nx).start(priority=1))

                @pl.when(nx + 1 >= nsteps - _NF)
                def _():
                    pl.when(nx + 1 < nsteps)(lambda: k_copy(nx + 1).start(priority=1))
            else:
                v_copy(nx).start(priority=1)

        def prefetch_k(step, c, guarded):
            def go():
                for j in range(c * _NPK // nch, (c + 1) * _NPK // nch):
                    k_piece(step + _LK, j).start()
            if guarded:
                pl.when(step + _LK < nsteps - _NF)(go)
            else:
                go()

        def attend(step, par, do_next, rd, wr, guarded=False):
            v_copy(step).wait()
            if do_next:
                k_wait(step + 1)
                prefetch_v(step, guarded)
            m = jnp.max(m_scr[par], axis=-1, keepdims=True)
            m_fin[rd] = jnp.broadcast_to(m, (M, 128))
            p = exp_chunk(par, 0, m_fin[rd])
            for c in range(nch):
                if do_next:
                    qk_chunk(step + 1, c, 1 - par, wr)
                p_next = exp_chunk(par, c + 1, m_fin[rd]) if c + 1 < nch else None
                pv_chunk(step, p, c)
                p = p_next
                if do_next:
                    prefetch_k(step, c, guarded)
            l = jnp.sum(l_scr[...], axis=-1, keepdims=True)
            return (pv_scr[...] / l).astype(jnp.bfloat16)

        def store_o(step, o):
            row = pl.multiple_of((step & (B - 1)) * SQ, SQ)
            for r in range(REP):
                o_scr[pl.ds(row, SQ), r * DH:(r + 1) * DH] = o[r * SQ:(r + 1) * SQ, :]

        def final_rows(b, o):
            row = pl.multiple_of(b * SQ, SQ)
            oc = jnp.concatenate([o[r * SQ:(r + 1) * SQ, :] for r in range(REP)], axis=1)
            part = lax.dot_general(oc, wo_v[lasth & 1], _NT,
                                   preferred_element_type=jnp.float32)
            out_v[b] = (acc[pl.ds(row, SQ), :] + part).astype(jnp.bfloat16)
            out_copy(b).start()

        x_copy = pltpu.make_async_copy(x_hbm, x_v, x_sem)
        x_copy.start()
        wq_copy(0).start()
        k_copy(0).start()
        acc[...] = jnp.zeros_like(acc)
        x_copy.wait()
        wq_copy(0).wait()
        wq_copy(1).start()
        for s in range(1, _LK):
            k_copy(s).start()
        for s in range(_LV):
            v_copy(s).start(priority=1)
        wo_copy(0).start()
        q_proj(0)
        k_wait(0)
        for c in range(nch):
            qk_chunk(0, c, 0)

        def group(h, carry):
            wq_copy(h + 1).wait()
            q_proj(h + 1)
            pl.when(h + 2 < HKV)(lambda: wq_copy(h + 2).start())
            wo_copy(h + 1).start()

            def pair(bu, c):
                rd, wr = c
                for u in range(2):
                    step = h * B + 2 * bu + u
                    store_o(step, attend(step, u, True, rd, wr))
                    rd, wr = wr, rd
                return (c[1], c[0])

            carry = lax.fori_loop(0, B // 2, pair, carry)
            wo_copy(h).wait()
            acc[...] += lax.dot_general(o_scr[...], wo_v[h & 1], _NT,
                                        preferred_element_type=jnp.float32)
            return carry

        carry = lax.fori_loop(0, HKV - 1, group, (jnp.int32(0), jnp.int32(1)))

        wo_copy(lasth).wait()

        def last_pair(bu, c):
            rd, wr = c
            for u in range(2):
                step = lasth * B + 2 * bu + u

                def run(step=step, u=u, rd=rd, wr=wr):
                    o = attend(step, u, True, rd, wr, guarded=True)
                    final_rows(step & (B - 1), o)

                if u == 0:
                    run()
                else:
                    pl.when(step < nsteps - 1)(run)
                rd, wr = wr, rd
            return (c[1], c[0])

        rd, wr = lax.fori_loop(0, B // 2, last_pair, carry)
        final_rows(B - 1, attend(nsteps - 1, 1, False, rd, wr))
        for b in range(B):
            out_copy(b).wait()

    hbm = pl.BlockSpec(memory_space=pltpu.MemorySpace.HBM)
    return pl.pallas_call(
        kernel,
        out_shape=jax.ShapeDtypeStruct((B, SQ, D), jnp.bfloat16),
        in_specs=[hbm] * 5,
        out_specs=hbm,
        scratch_shapes=[
            pltpu.VMEM((B, SQ, D), jnp.bfloat16),
            pltpu.VMEM((2, D, GW), jnp.bfloat16),
            pltpu.VMEM((2, D, GW), jnp.bfloat16),
            pltpu.VMEM((nbuf, SK, DH), jnp.bfloat16),
            pltpu.VMEM((nbuf, SK, DH), jnp.bfloat16),
            pltpu.VMEM((2 * B, M, DH), jnp.bfloat16),
            pltpu.VMEM((B * SQ, GW), jnp.bfloat16),
            pltpu.VMEM((B * SQ, D), jnp.float32),
            pltpu.VMEM((B, SQ, D), jnp.bfloat16),
            pltpu.VMEM((2, M, SK), jnp.float32),
            pltpu.VMEM((2, M, 128), jnp.float32),
            pltpu.VMEM((M, 128), jnp.float32),
            pltpu.VMEM((M, DH), jnp.float32),
            pltpu.VMEM((2, M, 128), jnp.float32),
            pltpu.SemaphoreType.DMA((nbuf,)),
            pltpu.SemaphoreType.DMA((nbuf,)),
            pltpu.SemaphoreType.DMA((2, 2)),
            pltpu.SemaphoreType.DMA(()),
            pltpu.SemaphoreType.DMA((B,)),
        ],
        compiler_params=pltpu.CompilerParams(vmem_limit_bytes=100 * 1024 * 1024,
                                             disable_bounds_checks=True),
    )(x, k_cache, v_cache, wq, wo.T)
```
